```python
import os as _os
_os.environ.setdefault("JAX_PLATFORMS", "cpu")
import jax
import jax.numpy as jnp

def _softmax(x, axis=-1):
    return jax.nn.softmax(x, axis=axis)
def _gelu(x):
    return jax.nn.gelu(x, approximate=True)
def _silu(x):
    return jax.nn.silu(x)
def _sigmoid(x):
    return jax.nn.sigmoid(x)
def _layernorm(x, axis=-1, eps=1e-5):
    m = jnp.mean(x, axis=axis, keepdims=True)
    v = jnp.var(x, axis=axis, keepdims=True)
    return (x - m) / jnp.sqrt(v + eps)
def _scatter_add(tgt, idx, src, axis=0):
    return tgt.at[idx].add(src)
def _segment_sum(src, seg, n):
    return jax.ops.segment_sum(src, seg, n)
class _Rng:
    def __init__(self, key):
        self._k = key
    def _next(self):
        self._k, sub = jax.random.split(self._k)
        return sub
    def normal(self, shape):
        return jax.random.normal(self._next(), shape, dtype=jnp.bfloat16)
    def randint(self, lo, hi, shape):
        return jax.random.randint(self._next(), shape, lo, hi, dtype=jnp.int32)
    def uniform(self, shape, lo=0.0, hi=1.0):
        return jax.random.uniform(self._next(), shape, jnp.bfloat16, lo, hi)
    def permutation(self, n):
        return jax.random.permutation(self._next(), n)


kernel_name = 'standalone__instancenorm__sampling'

def setup_inputs():
    _rng = _Rng(jax.random.key(int.from_bytes(__import__("os").urandom(4), "little")))
    _w = (lambda a: (lambda t: t.astype(jnp.bfloat16) if jnp.issubdtype(t.dtype, jnp.floating) else t)(jnp.asarray(a)))
    B, C, H, W = 16, 640, 16, 32
    return {
        "x": _w((lambda *s: _rng.normal(s) * 0.05)(B, C, H, W)),
        "g": _w((lambda *s: _rng.normal(s) * 0.05)(C) + 1.0),
        "b": _w((lambda *s: _rng.normal(s) * 0.05)(C)),
    }

def reference(x, g, b):
    mu = x.mean(axis=(-2, -1), keepdims=True)
    var = ((x - mu) * (x - mu)).mean(axis=(-2, -1), keepdims=True)
    xhat = (x - mu) / jnp.sqrt(var + 1e-5)
    return xhat * g.reshape(1, -1, 1, 1) + b.reshape(1, -1, 1, 1)
```

```python
import jax
import jax.numpy as jnp
import jax.experimental.pallas as pl
import jax.experimental.pallas.tpu as pltpu

_EPS = 1e-5
_LANES = 128
_GROUP = 4
_WRITE_AT = 14


@jax.jit
def pallas_standalone__instancenorm__sampling_kernel(
    x: jax.Array,
    g: jax.Array,
    b: jax.Array,
):
    B, C, H, W = x.shape
    n = H * W
    n_cblk = C // _LANES
    n_groups = B // _GROUP

    def kernel_function(x_hbm, g_hbm, b_hbm, o_hbm,
                        xbuf, obuf, gbuf, bbuf, rsem, gsem, wsem):
        def read(i):
            return pltpu.make_async_copy(x_hbm.at[i], xbuf.at[i], rsem.at[i])

        def start_write_group(grp):
            rows = pl.ds(grp * _GROUP, _GROUP)
            for h in range(H):
                pltpu.make_async_copy(
                    obuf.at[rows, h], o_hbm.at[rows, h], wsem.at[0]).start()

        g_copy = pltpu.make_async_copy(g_hbm, gbuf, gsem.at[0])
        b_copy = pltpu.make_async_copy(b_hbm, bbuf, gsem.at[1])
        g_copy.start()
        b_copy.start()

        def start_read(i, carry):
            read(i).start()
            return carry

        jax.lax.fori_loop(0, B, start_read, 0)

        g_copy.wait()
        b_copy.wait()
        gamma = jnp.concatenate(
            [gbuf[pl.ds(j, 1), :] for j in range(n_cblk)], axis=1
        ).astype(jnp.float32)
        beta = jnp.concatenate(
            [bbuf[pl.ds(j, 1), :] for j in range(n_cblk)], axis=1
        ).astype(jnp.float32)

        def body(i, carry):
            read(i).wait()
            for grp in range(n_groups):
                if _GROUP * (grp + 1) - 1 < _WRITE_AT:
                    pl.when(i == _WRITE_AT)(lambda grp=grp: start_write_group(grp))

            xf = xbuf[i].reshape(n, C).astype(jnp.float32)
            mean = jnp.sum(xf, axis=0, keepdims=True) * (1.0 / n)
            xc = xf - mean
            var = jnp.sum(xc * xc, axis=0, keepdims=True) * (1.0 / n)
            scale = jax.lax.rsqrt(var + _EPS) * gamma
            obuf[i] = (xc * scale + beta).astype(obuf.dtype).reshape(H, W, C)

            for grp in range(n_groups):
                last = _GROUP * (grp + 1) - 1
                if last >= _WRITE_AT:
                    pl.when(i == last)(lambda grp=grp: start_write_group(grp))
            return carry

        jax.lax.fori_loop(0, B, body, 0)
        pltpu.make_async_copy(obuf, obuf, wsem.at[0]).wait()

    x_nhwc = x.transpose(0, 2, 3, 1)
    any_spec = pl.BlockSpec(memory_space=pl.ANY)
    out = pl.pallas_call(
        kernel_function,
        in_specs=[any_spec, any_spec, any_spec],
        out_specs=any_spec,
        out_shape=jax.ShapeDtypeStruct((B, H, W, C), x.dtype),
        scratch_shapes=[
            pltpu.VMEM((B, H, W, C), x.dtype),
            pltpu.VMEM((B, H, W, C), x.dtype),
            pltpu.VMEM((n_cblk, _LANES), g.dtype),
            pltpu.VMEM((n_cblk, _LANES), b.dtype),
            pltpu.SemaphoreType.DMA((B,)),
            pltpu.SemaphoreType.DMA((2,)),
            pltpu.SemaphoreType.DMA((1,)),
        ],
        compiler_params=pltpu.CompilerParams(vmem_limit_bytes=64 * 1024 * 1024),
        name="instancenorm_nhwc",
    )(x_nhwc, g.reshape(n_cblk, _LANES), b.reshape(n_cblk, _LANES))
    return out.transpose(0, 3, 1, 2)
```

```python
import jax
import jax.numpy as jnp
import jax.experimental.pallas as pl
import jax.experimental.pallas.tpu as pltpu

_EPS = 1e-5
_LANES = 128
_WRITE_GROUPS = (5, 5, 6)
_SPLIT_H = 6


@jax.jit
def pallas_standalone__instancenorm__sampling_kernel(
    x: jax.Array,
    g: jax.Array,
    b: jax.Array,
):
    B, C, H, W = x.shape
    n = H * W
    n_cblk = C // _LANES
    last = B - 1
    group_start = [sum(_WRITE_GROUPS[:k]) for k in range(len(_WRITE_GROUPS))]
    group_end = [s + m for s, m in zip(group_start, _WRITE_GROUPS)]
    early = [k for k, e in enumerate(group_end) if e <= last - 1]
    late = [k for k in range(len(_WRITE_GROUPS)) if k not in early]
    assert group_end[-1] == B and C % _LANES == 0 and 0 < _SPLIT_H < H

    def kernel_function(x_hbm, g_hbm, b_hbm, o_hbm, xbuf, obuf, gbuf, bbuf, wsem):
        def start_write_group(k):
            rows = pl.ds(group_start[k], _WRITE_GROUPS[k])
            for h in range(H):
                pltpu.make_async_copy(
                    obuf.at[rows, h], o_hbm.at[rows, h], wsem.at[0]).start()

        def load_and_normalize(rsem, lsem, gsem):
            def read(i):
                return pltpu.make_async_copy(x_hbm.at[i], xbuf.at[i], rsem.at[i])

            def read_last(part):
                hs = pl.ds(0, _SPLIT_H) if part == 0 else pl.ds(_SPLIT_H, H - _SPLIT_H)
                return pltpu.make_async_copy(
                    x_hbm.at[last, hs], xbuf.at[last, hs], lsem.at[part])

            g_copy = pltpu.make_async_copy(g_hbm, gbuf, gsem.at[0])
            b_copy = pltpu.make_async_copy(b_hbm, bbuf, gsem.at[1])
            read(0).start()
            g_copy.start()
            b_copy.start()

            def start_read(i, carry):
                read(i).start()
                return carry

            jax.lax.fori_loop(1, last, start_read, 0)
            read_last(0).start()
            read_last(1).start()

            g_copy.wait()
            b_copy.wait()
            gamma = jnp.concatenate(
                [gbuf[pl.ds(j, 1), :] for j in range(n_cblk)], axis=1
            ).astype(jnp.float32)
            beta = jnp.concatenate(
                [bbuf[pl.ds(j, 1), :] for j in range(n_cblk)], axis=1
            ).astype(jnp.float32)

            def body(i, carry):
                @pl.when(i < last)
                def _():
                    read(i).wait()

                @pl.when(i == last - 1)
                def _():
                    read_last(0).wait()
                    for k in early:
                        start_write_group(k)

                @pl.when(i == last)
                def _():
                    read_last(1).wait()

                xf = xbuf[i].reshape(n, C).astype(jnp.float32)
                mean = jnp.sum(xf, axis=0, keepdims=True) * (1.0 / n)
                xc = xf - mean
                var = jnp.sum(xc * xc, axis=0, keepdims=True) * (1.0 / n)
                scale = jax.lax.rsqrt(var + _EPS) * gamma
                obuf[i] = (xc * scale + beta).astype(obuf.dtype).reshape(H, W, C)

                for k in late:
                    pl.when(i == group_end[k] - 1)(lambda k=k: start_write_group(k))
                return carry

            jax.lax.fori_loop(0, B, body, 0)

        pl.run_scoped(
            load_and_normalize,
            pltpu.SemaphoreType.DMA((last,)),
            pltpu.SemaphoreType.DMA((2,)),
            pltpu.SemaphoreType.DMA((2,)),
        )
        pltpu.make_async_copy(obuf, o_hbm, wsem.at[0]).wait()

    x_nhwc = x.transpose(0, 2, 3, 1)
    any_spec = pl.BlockSpec(memory_space=pl.ANY)
    out = pl.pallas_call(
        kernel_function,
        in_specs=[any_spec, any_spec, any_spec],
        out_specs=any_spec,
        out_shape=jax.ShapeDtypeStruct((B, H, W, C), x.dtype),
        scratch_shapes=[
            pltpu.VMEM((B, H, W, C), x.dtype),
            pltpu.VMEM((B, H, W, C), x.dtype),
            pltpu.VMEM((n_cblk, _LANES), g.dtype),
            pltpu.VMEM((n_cblk, _LANES), b.dtype),
            pltpu.SemaphoreType.DMA((1,)),
        ],
        compiler_params=pltpu.CompilerParams(vmem_limit_bytes=64 * 1024 * 1024),
        name="instancenorm_nhwc",
    )(x_nhwc, g.reshape(n_cblk, _LANES), b.reshape(n_cblk, _LANES))
    return out.transpose(0, 3, 1, 2)
```
